```python
import os as _os
_os.environ.setdefault("JAX_PLATFORMS", "cpu")
import jax
import jax.numpy as jnp

def _softmax(x, axis=-1):
    return jax.nn.softmax(x, axis=axis)
def _gelu(x):
    return jax.nn.gelu(x, approximate=True)
def _silu(x):
    return jax.nn.silu(x)
def _sigmoid(x):
    return jax.nn.sigmoid(x)
def _layernorm(x, axis=-1, eps=1e-5):
    m = jnp.mean(x, axis=axis, keepdims=True)
    v = jnp.var(x, axis=axis, keepdims=True)
    return (x - m) / jnp.sqrt(v + eps)
def _scatter_add(tgt, idx, src, axis=0):
    return tgt.at[idx].add(src)
def _segment_sum(src, seg, n):
    return jax.ops.segment_sum(src, seg, n)
class _Rng:
    def __init__(self, key):
        self._k = key
    def _next(self):
        self._k, sub = jax.random.split(self._k)
        return sub
    def normal(self, shape):
        return jax.random.normal(self._next(), shape, dtype=jnp.bfloat16)
    def randint(self, lo, hi, shape):
        return jax.random.randint(self._next(), shape, lo, hi, dtype=jnp.int32)
    def uniform(self, shape, lo=0.0, hi=1.0):
        return jax.random.uniform(self._next(), shape, jnp.bfloat16, lo, hi)
    def permutation(self, n):
        return jax.random.permutation(self._next(), n)


kernel_name = 'sequential_preLN__compressed_kv_cla__dense_activation_mish__decode'

def setup_inputs():
    _rng = _Rng(jax.random.key(int.from_bytes(__import__("os").urandom(4), "little")))
    _w = (lambda a: (lambda t: t.astype(jnp.bfloat16) if jnp.issubdtype(t.dtype, jnp.floating) else t)(jnp.asarray(a)))
    def _A_setup():
        B, H, Sq, Sk, D, M = 2, 32, 1, 8192, 128, 512
        Dc = 4 * D
        return {
            "x": _w((lambda *s: _rng.normal(s) * 0.05)(B, Sq, M)),
            "c_kv": _w((lambda *s: _rng.normal(s) * 0.8)(B, Sk, Dc)),
            "w_q": _w((lambda *s: _rng.normal(s) * 0.8)(M, H, D) * (M ** -0.5)),
            "w_uk": _w((lambda *s: _rng.normal(s) * 0.8)(Dc, H, D) * (Dc ** -0.5)),
            "w_uv": _w((lambda *s: _rng.normal(s) * 0.8)(Dc, H, D) * (Dc ** -0.5)),
            "w_o": _w((lambda *s: _rng.normal(s) * 0.8)(H, D, M) * ((H * D) ** -0.5)),
        }
    _A_in = _A_setup()

    def _B_setup():
        B, S, D, F = 2, 1, 512, 1792
        return {
            "x": _w((lambda *s: _rng.normal(s) * 0.05)(B, S, D)),
            "w1": _w((lambda *s: _rng.normal(s) * 0.4)(D, F) * (D ** -0.5)),
            "b1": _w((lambda *s: _rng.normal(s) * 0.05)(F)),
            "w2": _w((lambda *s: _rng.normal(s) * 0.05)(F, D) * (F ** -0.5)),
        }
    _B_in = _B_setup()

    return {
        "A_x": _A_in["x"],
        "A_c_kv": _A_in["c_kv"],
        "A_w_q": _A_in["w_q"],
        "A_w_uk": _A_in["w_uk"],
        "A_w_uv": _A_in["w_uv"],
        "A_w_o": _A_in["w_o"],
        "B_x": _B_in["x"],
        "B_w1": _B_in["w1"],
        "B_b1": _B_in["b1"],
        "B_w2": _B_in["w2"],
    }

def reference(A_x, A_c_kv, A_w_q, A_w_uk, A_w_uv, A_w_o, B_x, B_w1, B_b1, B_w2):
    def _A_ref(x, c_kv, w_q, w_uk, w_uv, w_o):
        B, Sq, M = x.shape[0], x.shape[1], x.shape[2]
        Sk = c_kv.shape[1]
        H, D = w_q.shape[1], w_q.shape[2]
        q = jnp.einsum("bqm,mhd->bhqd", x, w_q)
        k = jnp.einsum("bkc,chd->bhkd", c_kv, w_uk)
        v = jnp.einsum("bkc,chd->bhkd", c_kv, w_uv)
        scores = jnp.einsum("bhqd,bhkd->bhqk", q, k) * (D ** -0.5)
        off = Sk - Sq
        qi = jnp.arange(Sq)[:, None]
        kj = jnp.arange(Sk)[None, :]
        cmask = kj <= (qi + off)
        scores = jnp.where(cmask[None, None], scores, -1e9)
        p = _softmax(scores, axis=-1)
        ctx = jnp.einsum("bhqk,bhkd->bhqd", p, v)
        return jnp.einsum("bhqd,hdm->bqm", ctx, w_o)

    def _B_ref(x, w1, b1, w2):
        h = jnp.einsum("bsd,df->bsf", x, w1) + b1
        sp = jnp.log1p(jnp.exp(-jnp.abs(h))) + jnp.where(h > 0, h, jnp.zeros_like(h))
        act = h * jnp.tanh(sp)
        return jnp.einsum("bsf,fd->bsd", act, w2)

    x = A_x
    h = x + _A_ref(_layernorm(x, axis=-1), A_c_kv, A_w_q, A_w_uk, A_w_uv, A_w_o)
    h2 = h + _B_ref(_layernorm(h, axis=-1), B_w1, B_b1, B_w2)
    return h2
```

```python
import jax
import jax.numpy as jnp
from jax import lax
import jax.experimental.pallas as pl
import jax.experimental.pallas.tpu as pltpu

_F32 = jnp.float32
_BF16 = jnp.bfloat16
_NT = (((1,), (1,)), ((), ()))
_LANES = 128

_CKV_DMA_ROWS = 4096
_CKV_STEP_ROWS = 2048
_W2_TAIL_ROWS = (640, 128)


def _layernorm_rows(x, eps=1e-5):
    m = jnp.mean(x, axis=-1, keepdims=True)
    xc = x - m
    v = jnp.mean(xc * xc, axis=-1, keepdims=True)
    return xc / jnp.sqrt(v + eps)


def _stack_rows(rows, rows_per_item, total_rows):
    n = rows[0].shape[-1]
    r = lax.broadcasted_iota(jnp.int32, (total_rows, n), 0)
    out = jnp.broadcast_to(rows[-1], (total_rows, n))
    for i in range(len(rows) - 2, -1, -1):
        out = jnp.where(r < (i + 1) * rows_per_item, rows[i], out)
    return out


def _kernel(x_hbm, b1_hbm, wq_hbm, wuk_hbm, ckv_hbm, wuv_hbm, wo_hbm, w1_hbm, w2_hbm,
            o_ref,
            x_buf, b1_buf, wq_buf, wuk_buf, ckv_buf, wuv_buf, wo_buf, w1_buf, w2_buf, sems):
    B, Sk, Dc = ckv_buf.shape
    M, H, D = wq_buf.shape
    F = w1_buf.shape[1]
    G = _LANES
    R = B * H
    TD, TC = _CKV_DMA_ROWS, _CKV_STEP_ROWS
    scale = float(D) ** -0.5

    copies = []

    def add(src, dst):
        copies.append(pltpu.make_async_copy(src, dst, sems.at[len(copies)]))
        return len(copies) - 1

    x_id = add(x_hbm, x_buf)
    b1_id = add(b1_hbm, b1_buf)
    wq_id = add(wq_hbm, wq_buf)
    wuk_id = add(wuk_hbm, wuk_buf)
    ckv_id = {(i, b): add(ckv_hbm.at[b, pl.ds(i * TD, TD)], ckv_buf.at[b, pl.ds(i * TD, TD)])
              for i in range(Sk // TD) for b in range(B)}
    wuv_id = add(wuv_hbm, wuv_buf)
    wo_id = add(wo_hbm, wo_buf)
    w1_id = add(w1_hbm, w1_buf)
    w2_chunks = []
    off = 0
    for n in (F - sum(_W2_TAIL_ROWS),) + _W2_TAIL_ROWS:
        w2_chunks.append((off, n, add(w2_hbm.at[pl.ds(off, n)], w2_buf.at[pl.ds(off, n)])))
        off += n
    for c in copies:
        c.start()

    waited = set()

    def wait(i):
        if i not in waited:
            copies[i].wait()
            waited.add(i)

    rep = (lax.broadcasted_iota(jnp.int32, (G, G * H), 1) // H
           == lax.broadcasted_iota(jnp.int32, (G, G * H), 0)).astype(_BF16)
    diag = (lax.broadcasted_iota(jnp.int32, (R, G * H), 1) % H
            == lax.broadcasted_iota(jnp.int32, (R, G * H), 0) % H)

    def per_head_project(a_bf, w_buf, w_id):
        n_out = w_buf.shape[2]
        acc = jnp.zeros((R, n_out), _F32)
        for g in range(w_buf.shape[0] // G):
            a_rep = jnp.dot(a_bf[:, g * G:(g + 1) * G], rep, preferred_element_type=_F32)
            a_bd = jnp.where(diag, a_rep, 0.0).astype(_BF16)
            wait(w_id)
            w_g = w_buf[pl.ds(g * G, G)].reshape(G * H, n_out)
            acc = acc + jnp.dot(a_bd, w_g, preferred_element_type=_F32)
        return acc

    wait(x_id)
    x_all = x_buf[...].astype(_F32)
    x_rows = [x_all[b:b + 1] for b in range(B)]
    xn_bf = _layernorm_rows(_stack_rows(x_rows, H, R)).astype(_BF16)
    q_bf = per_head_project(xn_bf, wq_buf, wq_id).astype(_BF16)

    wait(wuk_id)
    q_lat = []
    for g in range(Dc // G):
        w_g = wuk_buf[pl.ds(g * G, G)].reshape(G * H, D)
        t = lax.dot_general(q_bf, w_g, _NT, preferred_element_type=_F32)
        t = jnp.where(diag, t * scale, 0.0).astype(_BF16)
        q_lat.append(lax.dot_general(t, rep, _NT, preferred_element_type=_F32).astype(_BF16))
    q_lat = jnp.concatenate(q_lat, axis=1)

    state = [(jnp.full((H, 1), -jnp.inf, _F32), jnp.zeros((H, 1), _F32), jnp.zeros((H, Dc), _F32))
             for _ in range(B)]
    for i in range(Sk // TC):
        for b in range(B):
            m_prev, l_prev, acc_prev = state[b]
            wait(ckv_id[(i * TC // TD, b)])
            c = ckv_buf[b, pl.ds(i * TC, TC), :]
            s = lax.dot_general(q_lat[b * H:(b + 1) * H], c, _NT,
                                preferred_element_type=_F32)
            m_new = jnp.maximum(m_prev, jnp.max(s, axis=1, keepdims=True))
            alpha = jnp.exp(m_prev - m_new)
            p = jnp.exp(s - m_new)
            l_new = alpha * l_prev + jnp.sum(p, axis=1, keepdims=True)
            acc = alpha * acc_prev + jnp.dot(p.astype(_BF16), c, preferred_element_type=_F32)
            state[b] = (m_new, l_new, acc)
    ctx_lat = jnp.concatenate([acc / l for (_, l, acc) in state], axis=0)

    ctx_bf = per_head_project(ctx_lat.astype(_BF16), wuv_buf, wuv_id).astype(_BF16)
    blk = (lax.broadcasted_iota(jnp.int32, (R, H * D), 1) // D
           == lax.broadcasted_iota(jnp.int32, (R, H * D), 0) % H)
    ctx_bd = jnp.where(blk, jnp.concatenate([ctx_bf] * H, axis=1), jnp.zeros((), _BF16))
    wait(wo_id)
    o_heads = jnp.dot(ctx_bd, wo_buf[...].reshape(H * D, M), preferred_element_type=_F32)
    h_rows = [x_rows[b] + jnp.sum(o_heads[b * H:(b + 1) * H], axis=0, keepdims=True)
              for b in range(B)]

    h_st = _stack_rows(h_rows, 1, 8)
    hn_bf = _layernorm_rows(h_st).astype(_BF16)
    wait(b1_id)
    wait(w1_id)
    z = (jnp.dot(hn_bf, w1_buf[...], preferred_element_type=_F32)
         + b1_buf[...].astype(_F32).reshape(1, F))
    sp = jnp.log1p(jnp.exp(-jnp.abs(z))) + jnp.maximum(z, 0.0)
    act = (z * jnp.tanh(sp)).astype(_BF16)
    y = h_st
    for (off, n, cid) in w2_chunks:
        wait(cid)
        y = y + jnp.dot(act[:, off:off + n], w2_buf[pl.ds(off, n), :], preferred_element_type=_F32)
    o_ref[...] = y[:B].astype(o_ref.dtype)
    assert len(waited) == len(copies)


@jax.jit
def pallas_sequential_preLN__compressed_kv_cla__dense_activation_mish__decode_kernel(
    A_x: jax.Array,
    A_c_kv: jax.Array,
    A_w_q: jax.Array,
    A_w_uk: jax.Array,
    A_w_uv: jax.Array,
    A_w_o: jax.Array,
    B_x: jax.Array,
    B_w1: jax.Array,
    B_b1: jax.Array,
    B_w2: jax.Array,
):
    del B_x
    B, Sq, M = A_x.shape
    _, Sk, Dc = A_c_kv.shape
    _, H, D = A_w_q.shape
    F = B_w1.shape[1]
    assert Sq == 1, "decode kernel: single query position"
    assert B <= 8 and D == _LANES and M % _LANES == 0 and Dc % _LANES == 0 and F % _LANES == 0
    assert Sk % _CKV_DMA_ROWS == 0 and _CKV_DMA_ROWS % _CKV_STEP_ROWS == 0
    assert F > sum(_W2_TAIL_ROWS)

    n_copies = 7 + B * (Sk // _CKV_DMA_ROWS) + 1 + len(_W2_TAIL_ROWS)
    hbm = pl.BlockSpec(memory_space=pl.ANY)
    out = pl.pallas_call(
        _kernel,
        out_shape=jax.ShapeDtypeStruct((B, M), A_x.dtype),
        in_specs=[hbm] * 9,
        out_specs=pl.BlockSpec(memory_space=pltpu.VMEM),
        scratch_shapes=[
            pltpu.VMEM((B, M), A_x.dtype),
            pltpu.VMEM(B_b1.shape, B_b1.dtype),
            pltpu.VMEM(A_w_q.shape, A_w_q.dtype),
            pltpu.VMEM(A_w_uk.shape, A_w_uk.dtype),
            pltpu.VMEM(A_c_kv.shape, A_c_kv.dtype),
            pltpu.VMEM(A_w_uv.shape, A_w_uv.dtype),
            pltpu.VMEM(A_w_o.shape, A_w_o.dtype),
            pltpu.VMEM(B_w1.shape, B_w1.dtype),
            pltpu.VMEM(B_w2.shape, B_w2.dtype),
            pltpu.SemaphoreType.DMA((n_copies,)),
        ],
        compiler_params=pltpu.CompilerParams(vmem_limit_bytes=64 * 1024 * 1024),
    )(A_x.reshape(B, M), B_b1, A_w_q, A_w_uk, A_c_kv, A_w_uv, A_w_o, B_w1, B_w2)
    return out.reshape(B, Sq, M)
```

```python
import jax
import jax.numpy as jnp
from jax import lax
import jax.experimental.pallas as pl
import jax.experimental.pallas.tpu as pltpu

_F32 = jnp.float32
_BF16 = jnp.bfloat16
_NT = (((1,), (1,)), ((), ()))
_LANES = 128

_CKV_DMA_ROWS = 4096
_CKV_STEP_ROWS = 2048
_W2_TAIL_ROWS = (640, 128)


def _plan(Sk, F):
    td = max(r for r in (_CKV_DMA_ROWS, 2048, 1024, 512, 256, 128) if Sk % r == 0)
    tc = min(td, _CKV_STEP_ROWS)
    tail = _W2_TAIL_ROWS if F > sum(_W2_TAIL_ROWS) else ()
    return td, tc, (F - sum(tail),) + tail


def _layernorm_rows(x, eps=1e-5):
    m = jnp.mean(x, axis=-1, keepdims=True)
    xc = x - m
    v = jnp.mean(xc * xc, axis=-1, keepdims=True)
    return xc / jnp.sqrt(v + eps)


def _stack_rows(rows, rows_per_item, total_rows):
    n = rows[0].shape[-1]
    r = lax.broadcasted_iota(jnp.int32, (total_rows, n), 0)
    out = jnp.broadcast_to(rows[-1], (total_rows, n))
    for i in range(len(rows) - 2, -1, -1):
        out = jnp.where(r < (i + 1) * rows_per_item, rows[i], out)
    return out


def _kernel(x_hbm, b1_hbm, wq_hbm, wuk_hbm, ckv_hbm, wuv_hbm, wo_hbm, w1_hbm, w2_hbm,
            o_ref,
            x_buf, b1_buf, wq_buf, wuk_buf, ckv_buf, wuv_buf, wo_buf, w1_buf, w2_buf, sems):
    B, Sk, Dc = ckv_buf.shape
    M, H, D = wq_buf.shape
    F = w1_buf.shape[1]
    G = _LANES
    R = B * H
    TD, TC, w2_rows = _plan(Sk, F)
    scale = float(D) ** -0.5

    copies = []

    def add(src, dst):
        copies.append(pltpu.make_async_copy(src, dst, sems.at[len(copies)]))
        return len(copies) - 1

    x_id = add(x_hbm, x_buf)
    b1_id = add(b1_hbm, b1_buf)
    wq_id = add(wq_hbm, wq_buf)
    wuk_id = add(wuk_hbm, wuk_buf)
    ckv_id = {(i, b): add(ckv_hbm.at[b, pl.ds(i * TD, TD)], ckv_buf.at[b, pl.ds(i * TD, TD)])
              for i in range(Sk // TD) for b in range(B)}
    wuv_id = add(wuv_hbm, wuv_buf)
    wo_id = add(wo_hbm, wo_buf)
    w1_id = add(w1_hbm, w1_buf)
    w2_chunks = []
    off = 0
    for n in w2_rows:
        w2_chunks.append((off, n, add(w2_hbm.at[pl.ds(off, n)], w2_buf.at[pl.ds(off, n)])))
        off += n
    for c in copies:
        c.start()

    waited = set()

    def wait(i):
        if i not in waited:
            copies[i].wait()
            waited.add(i)

    rep = (lax.broadcasted_iota(jnp.int32, (G, G * H), 1) // H
           == lax.broadcasted_iota(jnp.int32, (G, G * H), 0)).astype(_BF16)
    diag = (lax.broadcasted_iota(jnp.int32, (R, G * H), 1) % H
            == lax.broadcasted_iota(jnp.int32, (R, G * H), 0) % H)

    def per_head_project(a_bf, w_buf, w_id):
        n_out = w_buf.shape[2]
        acc = jnp.zeros((R, n_out), _F32)
        for g in range(w_buf.shape[0] // G):
            a_rep = jnp.dot(a_bf[:, g * G:(g + 1) * G], rep, preferred_element_type=_F32)
            a_bd = jnp.where(diag, a_rep, 0.0).astype(_BF16)
            wait(w_id)
            w_g = w_buf[pl.ds(g * G, G)].reshape(G * H, n_out)
            acc = acc + jnp.dot(a_bd, w_g, preferred_element_type=_F32)
        return acc

    wait(x_id)
    x_all = x_buf[...].astype(_F32)
    x_rows = [x_all[b:b + 1] for b in range(B)]
    xn_bf = _layernorm_rows(_stack_rows(x_rows, H, R)).astype(_BF16)
    q_bf = per_head_project(xn_bf, wq_buf, wq_id).astype(_BF16)

    wait(wuk_id)
    q_lat = []
    for g in range(Dc // G):
        w_g = wuk_buf[pl.ds(g * G, G)].reshape(G * H, D)
        t = lax.dot_general(q_bf, w_g, _NT, preferred_element_type=_F32)
        t = jnp.where(diag, t * scale, 0.0).astype(_BF16)
        q_lat.append(lax.dot_general(t, rep, _NT, preferred_element_type=_F32).astype(_BF16))
    q_lat = jnp.concatenate(q_lat, axis=1)

    state = [(jnp.full((H, 1), -jnp.inf, _F32), jnp.zeros((H, 1), _F32), jnp.zeros((H, Dc), _F32))
             for _ in range(B)]
    for i in range(Sk // TC):
        for b in range(B):
            m_prev, l_prev, acc_prev = state[b]
            wait(ckv_id[(i * TC // TD, b)])
            c = ckv_buf[b, pl.ds(i * TC, TC), :]
            s = lax.dot_general(q_lat[b * H:(b + 1) * H], c, _NT,
                                preferred_element_type=_F32)
            m_new = jnp.maximum(m_prev, jnp.max(s, axis=1, keepdims=True))
            alpha = jnp.exp(m_prev - m_new)
            p = jnp.exp(s - m_new)
            l_new = alpha * l_prev + jnp.sum(p, axis=1, keepdims=True)
            acc = alpha * acc_prev + jnp.dot(p.astype(_BF16), c, preferred_element_type=_F32)
            state[b] = (m_new, l_new, acc)
    ctx_lat = jnp.concatenate([acc / l for (_, l, acc) in state], axis=0)

    ctx_bf = per_head_project(ctx_lat.astype(_BF16), wuv_buf, wuv_id).astype(_BF16)
    blk = (lax.broadcasted_iota(jnp.int32, (R, H * D), 1) // D
           == lax.broadcasted_iota(jnp.int32, (R, H * D), 0) % H)
    ctx_bd = jnp.where(blk, jnp.concatenate([ctx_bf] * H, axis=1), jnp.zeros((), _BF16))
    wait(wo_id)
    o_heads = jnp.dot(ctx_bd, wo_buf[...].reshape(H * D, M), preferred_element_type=_F32)
    h_rows = [x_rows[b] + jnp.sum(o_heads[b * H:(b + 1) * H], axis=0, keepdims=True)
              for b in range(B)]

    h_st = _stack_rows(h_rows, 1, 8)
    hn_bf = _layernorm_rows(h_st).astype(_BF16)
    wait(b1_id)
    wait(w1_id)
    z = (jnp.dot(hn_bf, w1_buf[...], preferred_element_type=_F32)
         + b1_buf[...].astype(_F32).reshape(1, F))
    sp = jnp.log1p(jnp.exp(-jnp.abs(z))) + jnp.maximum(z, 0.0)
    act = (z * jnp.tanh(sp)).astype(_BF16)
    y = h_st
    for (off, n, cid) in w2_chunks:
        wait(cid)
        y = y + jnp.dot(act[:, off:off + n], w2_buf[pl.ds(off, n), :], preferred_element_type=_F32)
    o_ref[...] = y[:B].astype(o_ref.dtype)
    assert len(waited) == len(copies)


@jax.jit
def pallas_sequential_preLN__compressed_kv_cla__dense_activation_mish__decode_kernel(
    A_x: jax.Array,
    A_c_kv: jax.Array,
    A_w_q: jax.Array,
    A_w_uk: jax.Array,
    A_w_uv: jax.Array,
    A_w_o: jax.Array,
    B_x: jax.Array,
    B_w1: jax.Array,
    B_b1: jax.Array,
    B_w2: jax.Array,
):
    del B_x
    B, Sq, M = A_x.shape
    _, Sk, Dc = A_c_kv.shape
    _, H, D = A_w_q.shape
    F = B_w1.shape[1]
    assert Sq == 1, "decode kernel: single query position"
    assert B <= 8 and D == _LANES and M % _LANES == 0 and Dc % _LANES == 0 and F % _LANES == 0
    assert Sk % _LANES == 0

    td, _, w2_rows = _plan(Sk, F)
    n_copies = 7 + B * (Sk // td) + len(w2_rows)
    hbm = pl.BlockSpec(memory_space=pl.ANY)
    out = pl.pallas_call(
        _kernel,
        out_shape=jax.ShapeDtypeStruct((B, M), A_x.dtype),
        in_specs=[hbm] * 9,
        out_specs=pl.BlockSpec(memory_space=pltpu.VMEM),
        scratch_shapes=[
            pltpu.VMEM((B, M), A_x.dtype),
            pltpu.VMEM(B_b1.shape, B_b1.dtype),
            pltpu.VMEM(A_w_q.shape, A_w_q.dtype),
            pltpu.VMEM(A_w_uk.shape, A_w_uk.dtype),
            pltpu.VMEM(A_c_kv.shape, A_c_kv.dtype),
            pltpu.VMEM(A_w_uv.shape, A_w_uv.dtype),
            pltpu.VMEM(A_w_o.shape, A_w_o.dtype),
            pltpu.VMEM(B_w1.shape, B_w1.dtype),
            pltpu.VMEM(B_w2.shape, B_w2.dtype),
            pltpu.SemaphoreType.DMA((n_copies,)),
        ],
        compiler_params=pltpu.CompilerParams(vmem_limit_bytes=64 * 1024 * 1024),
    )(A_x.reshape(B, M), B_b1, A_w_q, A_w_uk, A_c_kv, A_w_uv, A_w_o, B_w1, B_w2)
    return out.reshape(B, Sq, M)
```
